```python
import os as _os
_os.environ.setdefault("JAX_PLATFORMS", "cpu")
import jax
import jax.numpy as jnp

def _softmax(x, axis=-1):
    return jax.nn.softmax(x, axis=axis)
def _gelu(x):
    return jax.nn.gelu(x, approximate=True)
def _silu(x):
    return jax.nn.silu(x)
def _sigmoid(x):
    return jax.nn.sigmoid(x)
def _layernorm(x, axis=-1, eps=1e-5):
    m = jnp.mean(x, axis=axis, keepdims=True)
    v = jnp.var(x, axis=axis, keepdims=True)
    return (x - m) / jnp.sqrt(v + eps)
def _scatter_add(tgt, idx, src, axis=0):
    return tgt.at[idx].add(src)
def _segment_sum(src, seg, n):
    return jax.ops.segment_sum(src, seg, n)
class _Rng:
    def __init__(self, key):
        self._k = key
    def _next(self):
        self._k, sub = jax.random.split(self._k)
        return sub
    def normal(self, shape):
        return jax.random.normal(self._next(), shape, dtype=jnp.bfloat16)
    def randint(self, lo, hi, shape):
        return jax.random.randint(self._next(), shape, lo, hi, dtype=jnp.int32)
    def uniform(self, shape, lo=0.0, hi=1.0):
        return jax.random.uniform(self._next(), shape, jnp.bfloat16, lo, hi)
    def permutation(self, n):
        return jax.random.permutation(self._next(), n)


kernel_name = 'standalone__gqa_block_cached__near_ridge'

def setup_inputs():
    _rng = _Rng(jax.random.key(int.from_bytes(__import__("os").urandom(4), "little")))
    _w = (lambda a: (lambda t: t.astype(jnp.bfloat16) if jnp.issubdtype(t.dtype, jnp.floating) else t)(jnp.asarray(a)))
    B, Sq, D = 32, 112, 448
    Hq, Hkv, Sk, Dh = 16, 8, 512, 256
    assert Hq % Hkv == 0, (Hq, Hkv)
    return {
        "x": _w((lambda *s: _rng.normal(s) * 0.8)(B, Sq, D)),
        "k_cache": _w((lambda *s: _rng.normal(s) * 0.8)(B, Hkv, Sk, Dh)),
        "v_cache": _w((lambda *s: _rng.normal(s) * 0.05)(B, Hkv, Sk, Dh)),
        "wq": _w((lambda *s: _rng.normal(s) * 0.8)(D, Hq * Dh) * (D ** -0.5)),
        "wo": _w((lambda *s: _rng.normal(s) * 0.05)(Hq * Dh, D) * ((Hq * Dh) ** -0.5)),
    }

def reference(x, k_cache, v_cache, wq, wo):
    B, Sq, D = x.shape
    Hq, Dh = 16, 256
    Hkv = k_cache.shape[1]
    rep = Hq // Hkv
    q = (lambda x, *d: x.transpose(*d))((x @ wq).reshape(B, Sq, Hq, Dh), 0, 2, 1, 3)
    k = jnp.repeat(k_cache, rep, axis=1)
    v = jnp.repeat(v_cache, rep, axis=1)
    scores = jnp.einsum("bhqd,bhkd->bhqk", q, k) * (Dh ** -0.5)
    p = _softmax(scores, axis=-1)
    o = jnp.einsum("bhqk,bhkd->bhqd", p, v)
    return (lambda x, *d: x.transpose(*d))(o, 0, 2, 1, 3).reshape(B, Sq, Hq * Dh) @ wo
```

```python
import functools

import jax
import jax.numpy as jnp
import jax.experimental.pallas as pl
import jax.experimental.pallas.tpu as pltpu


def _kernel(x_ref, k_ref, v_ref, wq_ref, wo_ref, o_ref, acc_ref, *, bb, sq, rep, dh, scale):
    h = pl.program_id(1)
    nh = pl.num_programs(1)
    d = x_ref.shape[-1]

    x = x_ref[...].reshape(bb * sq, d)
    q = jnp.dot(x, wq_ref[...], preferred_element_type=jnp.float32)
    q = (q.astype(jnp.bfloat16) * scale).astype(jnp.bfloat16)

    outs = []
    for b in range(bb):
        qb = q[b * sq:(b + 1) * sq]
        q2 = jnp.concatenate([qb[:, r * dh:(r + 1) * dh] for r in range(rep)], axis=0)
        k = k_ref[b, 0]
        v = v_ref[b, 0]
        s = jax.lax.dot_general(q2, k, (((1,), (1,)), ((), ())),
                                preferred_element_type=jnp.float32)
        m = jnp.max(s, axis=-1, keepdims=True)
        p = jnp.exp(s - m)
        l = jnp.sum(p, axis=-1, keepdims=True)
        o = jnp.dot(p.astype(jnp.bfloat16), v, preferred_element_type=jnp.float32)
        o = (o / l).astype(jnp.bfloat16)
        outs.append(jnp.concatenate([o[r * sq:(r + 1) * sq] for r in range(rep)], axis=1))
    o_all = jnp.concatenate(outs, axis=0)
    contrib = jnp.dot(o_all, wo_ref[...], preferred_element_type=jnp.float32)

    @pl.when(h == 0)
    def _():
        acc_ref[...] = contrib

    @pl.when(h > 0)
    def _():
        acc_ref[...] += contrib

    @pl.when(h == nh - 1)
    def _():
        o_ref[...] = acc_ref[...].reshape(bb, sq, d).astype(o_ref.dtype)


@jax.jit
def pallas_standalone__gqa_block_cached__near_ridge_kernel(
    x: jax.Array,
    k_cache: jax.Array,
    v_cache: jax.Array,
    wq: jax.Array,
    wo: jax.Array,
):
    B, Sq, D = x.shape
    _, Hkv, Sk, Dh = k_cache.shape
    Hq = wq.shape[1] // Dh
    rep = Hq // Hkv
    bb = 4
    scale = Dh ** -0.5

    kernel = functools.partial(_kernel, bb=bb, sq=Sq, rep=rep, dh=Dh, scale=scale)
    return pl.pallas_call(
        kernel,
        grid=(B // bb, Hkv),
        in_specs=[
            pl.BlockSpec((bb, Sq, D), lambda b, h: (b, 0, 0)),
            pl.BlockSpec((bb, 1, Sk, Dh), lambda b, h: (b, h, 0, 0)),
            pl.BlockSpec((bb, 1, Sk, Dh), lambda b, h: (b, h, 0, 0)),
            pl.BlockSpec((D, rep * Dh), lambda b, h: (0, h)),
            pl.BlockSpec((rep * Dh, D), lambda b, h: (h, 0)),
        ],
        out_specs=pl.BlockSpec((bb, Sq, D), lambda b, h: (b, 0, 0)),
        out_shape=jax.ShapeDtypeStruct((B, Sq, D), x.dtype),
        scratch_shapes=[pltpu.VMEM((bb * Sq, D), jnp.float32)],
        compiler_params=pltpu.CompilerParams(
            dimension_semantics=("arbitrary", "arbitrary"),
            vmem_limit_bytes=100 * 1024 * 1024,
        ),
    )(x, k_cache, v_cache, wq, wo)
```

```python
import functools


import jax
import jax.numpy as jnp
from jax import lax
import jax.experimental.pallas as pl
import jax.experimental.pallas.tpu as pltpu

U = 2
NW0 = 2
LOG2E = 1.4426950408889634
NT = (((1,), (1,)), ((), ()))
LANES = 128


def _kernel(x_hbm, k_hbm, v_hbm, wq_hbm, wot_hbm, out_hbm,
            xbuf, kbuf, vbuf, wqbuf, wobuf, qbuf, acc_ref, obuf,
            xsem, ksem, vsem, wqsem, wosem, osem,
            *, bb, sq, rep, dh, nh, nb, qscale):
    npb = nh // U
    bi = pl.program_id(0)
    ph = pl.program_id(1)
    m = bb * sq
    cw = rep * dh
    ntile = m // LANES

    def kv_copy(hbm, buf, sem, blk, hp, slot, u):
        return pltpu.make_async_copy(
            hbm.at[pl.ds(blk * bb, bb), hp * U + u], buf.at[slot, u], sem.at[slot, u])

    k_copy = functools.partial(kv_copy, k_hbm, kbuf, ksem)
    v_copy = functools.partial(kv_copy, v_hbm, vbuf, vsem)

    def start_kv(blk, hp, slot):
        for u in range(U):
            k_copy(blk, hp, slot, u).start()
            v_copy(blk, hp, slot, u).start()

    def x_copy(blk):
        slot = lax.rem(blk, 2)
        return pltpu.make_async_copy(
            x_hbm.at[pl.ds(blk * m, m)], xbuf.at[slot], xsem.at[slot])

    def wq_copy(hh):
        return pltpu.make_async_copy(
            wq_hbm.at[:, pl.ds(hh * cw, cw)], wqbuf.at[hh], wqsem.at[hh])

    def wo_copy(hh):
        return pltpu.make_async_copy(
            wot_hbm.at[:, pl.ds(hh * cw, cw)], wobuf.at[hh], wosem.at[hh])

    def o_copy(blk):
        return pltpu.make_async_copy(
            obuf, out_hbm.at[pl.ds(blk * m, m)], osem.at[0])

    def qproj(x, h):
        q = jnp.dot(x, wqbuf[h], preferred_element_type=jnp.float32)
        qbuf[h] = (q * qscale).astype(qbuf.dtype)

    first_step = jnp.logical_and(bi == 0, ph == 0)

    @pl.when(first_step)
    def _():
        x_copy(0).start()
        for h in range(NW0):
            wq_copy(h).start()
        acc_ref[...] = jnp.zeros_like(acc_ref)
        for h in range(NW0):
            wq_copy(h).wait()

    @pl.when(ph == 0)
    def _():
        x_copy(bi).wait()

        @pl.when(bi > 1)
        def _():
            o_copy(bi - 2).wait()

        @pl.when(bi == 0)
        def _():
            for h in range(NW0, nh):
                wq_copy(h).start()
            start_kv(0, 0, 0)
            for u in range(U):
                wo_copy(u).start()

        x = xbuf[lax.rem(bi, 2)]
        qproj(x, 0)
        obuf[...] = acc_ref[...].T.astype(obuf.dtype)
        acc_ref[...] = jnp.zeros_like(acc_ref)

        @pl.when(bi > 0)
        def _():
            o_copy(bi - 1).start()
        for h in range(1, nh):
            if h == NW0:
                @pl.when(bi == 0)
                def _():
                    for hh in range(NW0, nh):
                        wq_copy(hh).wait()
            qproj(x, h)

    @pl.when(ph > 0)
    def _():
        hp = ph - 1
        slot = lax.rem(hp, 2)

        @pl.when(bi == 0)
        def _():
            for u in range(U):
                wo_copy(hp * U + u).wait()
        for u in range(U):
            k_copy(bi, hp, slot, u).wait()
            v_copy(bi, hp, slot, u).wait()

        last_pair = hp == npb - 1
        nblk = jnp.where(last_pair, bi + 1, bi)
        nhp = jnp.where(last_pair, 0, hp + 1)

        @pl.when(nblk < nb)
        def _():
            start_kv(nblk, nhp, 1 - slot)

        @pl.when(jnp.logical_and(bi == 0, hp + 1 < npb))
        def _():
            for u in range(U):
                wo_copy((hp + 1) * U + u).start()

        @pl.when(jnp.logical_and(hp == 0, bi + 1 < nb))
        def _():
            x_copy(bi + 1).start()

        for u in range(U):
            h = hp * U + u

            def qk(b):
                q2 = jnp.concatenate(
                    [qbuf[h, b * sq:(b + 1) * sq, r * dh:(r + 1) * dh] for r in range(rep)],
                    axis=0)
                return lax.dot_general(q2, kbuf[slot, u, b], NT,
                                       preferred_element_type=jnp.float32)

            def pv(b, s):
                mx = jnp.max(s, axis=-1, keepdims=True)
                p = jnp.exp2(s - mx)
                l = jnp.sum(p, axis=-1, keepdims=True)
                o = jnp.dot(p.astype(jnp.bfloat16), vbuf[slot, u, b],
                            preferred_element_type=jnp.float32)
                o = o * pl.reciprocal(l, approx=False, full_range=False)
                o = o.astype(jnp.bfloat16)
                return jnp.concatenate([o[r * sq:(r + 1) * sq] for r in range(rep)], axis=1)

            outs = []

            def rows(lo, hi):
                parts = []
                for b in range(lo // sq, (hi - 1) // sq + 1):
                    a = max(lo, b * sq) - b * sq
                    e = min(hi, (b + 1) * sq) - b * sq
                    parts.append(outs[b][a:e])
                return parts[0] if len(parts) == 1 else jnp.concatenate(parts, axis=0)

            def oproj(j):
                lo, hi = j * LANES, (j + 1) * LANES
                acc_ref[:, lo:hi] += lax.dot_general(
                    wobuf[h], rows(lo, hi), NT, preferred_element_type=jnp.float32)

            s_next = qk(0)
            for b in range(bb):
                s_cur = s_next
                if b + 1 < bb:
                    s_next = qk(b + 1)
                outs.append(pv(b, s_cur))
                if b >= 2:
                    oproj(b - 2)
            oproj(ntile - 1)

    @pl.when(jnp.logical_and(bi == nb - 1, ph == npb))
    def _():
        o_copy(nb - 2).wait()
        for j in range(ntile):
            lo, hi = j * LANES, (j + 1) * LANES
            obuf[lo:hi, :] = acc_ref[:, lo:hi].T.astype(obuf.dtype)
            pltpu.make_async_copy(
                obuf.at[pl.ds(lo, LANES)],
                out_hbm.at[pl.ds((nb - 1) * m + lo, LANES)], osem.at[0]).start()
        o_copy(nb - 1).wait()


@jax.jit
def pallas_standalone__gqa_block_cached__near_ridge_kernel(
    x: jax.Array,
    k_cache: jax.Array,
    v_cache: jax.Array,
    wq: jax.Array,
    wo: jax.Array,
):
    B, Sq, D = x.shape
    _, Hkv, Sk, Dh = k_cache.shape
    Hq = wq.shape[1] // Dh
    rep = Hq // Hkv
    bb = 8
    nb = B // bb
    m = bb * Sq
    cw = rep * Dh
    qscale = (Dh ** -0.5) * LOG2E

    kernel = functools.partial(_kernel, bb=bb, sq=Sq, rep=rep, dh=Dh, nh=Hkv, nb=nb,
                               qscale=qscale)
    hbm = pl.BlockSpec(memory_space=pltpu.HBM)
    out = pl.pallas_call(
        kernel,
        grid=(nb, Hkv // U + 1),
        in_specs=[hbm] * 5,
        out_specs=hbm,
        out_shape=jax.ShapeDtypeStruct((B * Sq, D), x.dtype),
        scratch_shapes=[
            pltpu.VMEM((2, m, D), x.dtype),
            pltpu.VMEM((2, U, bb, Sk, Dh), k_cache.dtype),
            pltpu.VMEM((2, U, bb, Sk, Dh), v_cache.dtype),
            pltpu.VMEM((Hkv, D, cw), wq.dtype),
            pltpu.VMEM((Hkv, D, cw), wo.dtype),
            pltpu.VMEM((Hkv, m, cw), x.dtype),
            pltpu.VMEM((D, m), jnp.float32),
            pltpu.VMEM((m, D), x.dtype),
            pltpu.SemaphoreType.DMA((2,)),
            pltpu.SemaphoreType.DMA((2, U)),
            pltpu.SemaphoreType.DMA((2, U)),
            pltpu.SemaphoreType.DMA((Hkv,)),
            pltpu.SemaphoreType.DMA((Hkv,)),
            pltpu.SemaphoreType.DMA((1,)),
        ],
        compiler_params=pltpu.CompilerParams(
            dimension_semantics=("arbitrary", "arbitrary"),
            vmem_limit_bytes=100 * 1024 * 1024,
            disable_bounds_checks=True,
        ),
    )(x.reshape(B * Sq, D), k_cache, v_cache, wq, wo.T)
    return out.reshape(B, Sq, D)
```

```python
import functools

import jax
import jax.numpy as jnp
from jax import lax
import jax.experimental.pallas as pl
import jax.experimental.pallas.tpu as pltpu

U = 2
LANES = 128
LOG2E = 1.4426950408889634
NT = (((1,), (1,)), ((), ()))


def _kernel(x_hbm, k_hbm, v_hbm, wq_hbm, wot_hbm, out_hbm,
            xbuf, kvbuf, wqbuf, wobuf, qbuf, acc_ref, obuf,
            xsem, x0sem, kvsem, wqsem, wosem, osem,
            *, bb, sq, rep, dh, nh, nb, qscale):
    npb = nh // U
    m = bb * sq
    cw = rep * dh
    ntile = m // LANES
    assert npb >= 4 and npb & (npb - 1) == 0 and nb >= 2

    def start_kv(blk, hp, slot):
        for u in range(U):
            for t, hbm in enumerate((k_hbm, v_hbm)):
                pltpu.make_async_copy(
                    hbm.at[pl.ds(blk * bb, bb), hp * U + u], kvbuf.at[slot, t, u],
                    kvsem.at[slot]).start()

    def wait_kv(slot):
        pltpu.make_async_copy(kvbuf.at[slot], kvbuf.at[slot], kvsem.at[slot]).wait()

    def x_copy(blk):
        slot = blk & 1
        return pltpu.make_async_copy(
            x_hbm.at[pl.ds(blk * m, m)], xbuf.at[slot], xsem.at[slot])

    def x0_copy(half):
        mh = m // 2
        return pltpu.make_async_copy(
            x_hbm.at[pl.ds(half * mh, mh)], xbuf.at[0, pl.ds(half * mh, mh)],
            x0sem.at[half])

    def wq_copy(h):
        return pltpu.make_async_copy(
            wq_hbm.at[:, pl.ds(h * cw, cw)], wqbuf.at[h], wqsem.at[h])

    def wo_copy(h):
        return pltpu.make_async_copy(
            wot_hbm.at[:, pl.ds(h * cw, cw)], wobuf.at[h], wosem.at[h])

    def tile_out(blk, t, buf):
        return pltpu.make_async_copy(
            obuf.at[buf, pl.ds(t * LANES, LANES)],
            out_hbm.at[pl.ds(blk * m + t * LANES, LANES)], osem.at[0])

    def wait_out():
        pltpu.make_async_copy(obuf.at[0], out_hbm.at[pl.ds(0, m)], osem.at[0]).wait()

    def project(x, w):
        q = jnp.dot(x, w, preferred_element_type=jnp.float32)
        return (q * qscale).astype(qbuf.dtype)

    x0_copy(0).start()
    wq_copy(0).start()
    x0_copy(1).start()
    wq_copy(1).start()
    acc_ref[...] = jnp.zeros_like(acc_ref)
    x0_copy(0).wait()
    wq_copy(0).wait()
    for h in range(U, nh):
        wq_copy(h).start()
    start_kv(0, 0, 0)
    for u in range(U):
        wo_copy(u).start()
    x_copy(1).start()
    qbuf[0, :m // 2] = project(xbuf[0, :m // 2], wqbuf[0])
    x0_copy(1).wait()
    wq_copy(1).wait()
    qbuf[0, m // 2:] = project(xbuf[0, m // 2:], wqbuf[0])
    qbuf[1] = project(xbuf[0], wqbuf[1])

    def first_projection(p, carry):
        for u in range(U):
            wq_copy(p * U + u).wait()
        wq_pair = wqbuf.at[pl.ds(p * U, U)]
        q_pair = qbuf.at[pl.ds(p * U, U)]
        for u in range(U):
            q_pair[u] = project(xbuf[0], wq_pair[u])
        return carry

    lax.fori_loop(1, npb, first_projection, 0)

    def step(g, last_block):
        if last_block:
            bi = nb - 1
            hp = g
        else:
            bi = lax.shift_right_logical(g, npb.bit_length() - 1)
            hp = g & (npb - 1)
        slot = hp & 1
        first_pair = hp == 0
        last_pair = hp == npb - 1

        if not last_block:
            @pl.when(bi == 0)
            def _():
                for u in range(U):
                    wo_copy(hp * U + u).wait()

            @pl.when(first_pair)
            def _():
                x_copy(bi + 1).wait()

        @pl.when(jnp.logical_and(hp == 2, bi > 0))
        def _():
            wait_out()
        wait_kv(slot)

        def prefetch():
            nblk = jnp.where(last_pair, bi + 1, bi)
            nhp = jnp.where(last_pair, 0, hp + 1)

            @pl.when(nblk < nb)
            def _():
                start_kv(nblk, nhp, 1 - slot)

            if not last_block:
                @pl.when(jnp.logical_and(bi == 0, hp + 1 < npb))
                def _():
                    for u in range(U):
                        wo_copy((hp + 1) * U + u).start()

                @pl.when(jnp.logical_and(first_pair, bi + 2 < nb))
                def _():
                    x_copy(bi + 2).start()

        wq_pair = wqbuf.at[pl.ds(hp * U, U)]
        wo_pair = wobuf.at[pl.ds(hp * U, U)]
        q_pair = qbuf.at[pl.ds(hp * U, U)]
        k_all = kvbuf.at[slot, 0]
        v_all = kvbuf.at[slot, 1]

        for u in range(U):
            def qk(b):
                q2 = jnp.concatenate(
                    [q_pair[u, b * sq:(b + 1) * sq, r * dh:(r + 1) * dh]
                     for r in range(rep)], axis=0)
                return lax.dot_general(q2, k_all[u, b], NT,
                                       preferred_element_type=jnp.float32)

            def pv(b, s):
                mx = jnp.max(s, axis=-1, keepdims=True)
                p = jnp.exp2(s - mx)
                l = jnp.sum(p, axis=-1, keepdims=True)
                o = jnp.dot(p.astype(jnp.bfloat16), v_all[u, b],
                            preferred_element_type=jnp.float32)
                o = o * pl.reciprocal(l, approx=False, full_range=False)
                o = o.astype(jnp.bfloat16)
                return jnp.concatenate([o[r * sq:(r + 1) * sq] for r in range(rep)], axis=1)

            outs = []

            def rows(lo, hi):
                parts = []
                for b in range(lo // sq, (hi - 1) // sq + 1):
                    a = max(lo, b * sq) - b * sq
                    e = min(hi, (b + 1) * sq) - b * sq
                    parts.append(outs[b][a:e])
                return parts[0] if len(parts) == 1 else jnp.concatenate(parts, axis=0)

            def oproj(j):
                lo, hi = j * LANES, (j + 1) * LANES
                prev = acc_ref[j]
                if u == 0:
                    obuf[slot, lo:hi, :] = prev.T.astype(obuf.dtype)

                    @pl.when(jnp.logical_and(first_pair, bi > 0))
                    def _():
                        tile_out(bi - 1, j, 0).start()
                    prev = jnp.where(first_pair, 0.0, prev)
                new = prev + lax.dot_general(wo_pair[u], rows(lo, hi), NT,
                                             preferred_element_type=jnp.float32)
                acc_ref[j] = new
                if last_block and u == U - 1 and j < ntile - 1:
                    obuf[2, lo:hi, :] = new.T.astype(obuf.dtype)

                    @pl.when(last_pair)
                    def _():
                        tile_out(nb - 1, j, 2).start()

            s_next = qk(0)
            emitted = 0
            for b in range(bb):
                s_cur = s_next
                if b + 1 < bb:
                    s_next = qk(b + 1)
                if u == 0 and b == 1:
                    prefetch()
                if not last_block and b == bb - 1:
                    q_pair[u] = project(xbuf[(bi + 1) & 1], wq_pair[u])
                outs.append(pv(b, s_cur))
                while (emitted + 1) * LANES <= b * sq:
                    oproj(emitted)
                    emitted += 1
            while emitted < ntile:
                oproj(emitted)
                emitted += 1

    def inner_step(g, carry):
        step(g, False)
        return carry

    def last_block_step(g, carry):
        step(g, True)
        return carry

    lax.fori_loop(0, (nb - 1) * npb, inner_step, 0)
    lax.fori_loop(0, npb, last_block_step, 0)

    t = ntile - 1
    obuf[2, t * LANES:(t + 1) * LANES, :] = acc_ref[t].T.astype(obuf.dtype)
    tile_out(nb - 1, t, 2).start()
    wait_out()


@jax.jit
def pallas_standalone__gqa_block_cached__near_ridge_kernel(
    x: jax.Array,
    k_cache: jax.Array,
    v_cache: jax.Array,
    wq: jax.Array,
    wo: jax.Array,
):
    B, Sq, D = x.shape
    _, Hkv, Sk, Dh = k_cache.shape
    Hq = wq.shape[1] // Dh
    rep = Hq // Hkv
    bb = 8
    nb = B // bb
    m = bb * Sq
    cw = rep * Dh
    assert B % bb == 0 and m % LANES == 0 and Hkv % U == 0
    qscale = (Dh ** -0.5) * LOG2E

    kernel = functools.partial(_kernel, bb=bb, sq=Sq, rep=rep, dh=Dh, nh=Hkv, nb=nb,
                               qscale=qscale)
    hbm = pl.BlockSpec(memory_space=pltpu.HBM)
    out = pl.pallas_call(
        kernel,
        in_specs=[hbm] * 5,
        out_specs=hbm,
        out_shape=jax.ShapeDtypeStruct((B * Sq, D), x.dtype),
        scratch_shapes=[
            pltpu.VMEM((2, m, D), x.dtype),
            pltpu.VMEM((2, 2, U, bb, Sk, Dh), k_cache.dtype),
            pltpu.VMEM((Hkv, D, cw), wq.dtype),
            pltpu.VMEM((Hkv, D, cw), wo.dtype),
            pltpu.VMEM((Hkv, m, cw), x.dtype),
            pltpu.VMEM((m // LANES, D, LANES), jnp.float32),
            pltpu.VMEM((3, m, D), x.dtype),
            pltpu.SemaphoreType.DMA((2,)),
            pltpu.SemaphoreType.DMA((2,)),
            pltpu.SemaphoreType.DMA((2,)),
            pltpu.SemaphoreType.DMA((Hkv,)),
            pltpu.SemaphoreType.DMA((Hkv,)),
            pltpu.SemaphoreType.DMA((1,)),
        ],
        compiler_params=pltpu.CompilerParams(
            vmem_limit_bytes=100 * 1024 * 1024,
            disable_bounds_checks=True,
        ),
    )(x.reshape(B * Sq, D), k_cache, v_cache, wq, wo.T)
    return out.reshape(B, Sq, D)
```

```python
import functools

import jax
import jax.numpy as jnp
from jax import lax
import jax.experimental.pallas as pl
import jax.experimental.pallas.tpu as pltpu

U = 2
LANES = 128
LOG2E = 1.4426950408889634
NT = (((1,), (1,)), ((), ()))


def _schedule(bb, sq, ntile, last_block):
    lag = 4 if last_block else 2
    n = U * bb
    ops = [("qk", 0, 0)]
    todo = [(u, j) for u in range(U) for j in range(ntile)]
    for i in range(n):
        u, b = divmod(i, bb)
        if i + 1 < n:
            ops.append(("qk",) + divmod(i + 1, bb))
        if i == 1:
            ops.append(("prefetch",))
        if not last_block and b == bb - 1:
            ops.append(("project", u))
        ops.append(("pv", u, b))
        while todo:
            tu, tj = todo[0]
            last_producer = tu * bb + ((tj + 1) * LANES - 1) // sq
            if last_producer + lag > i and i < n - 1:
                break
            ops.append(("out", tu, tj))
            todo.pop(0)
    return ops


def _kernel(x_hbm, k_hbm, v_hbm, wq_hbm, wot_hbm, out_hbm,
            xbuf, kvbuf, wqbuf, wobuf, qbuf, acc_ref, obuf,
            xsem, x0sem, kvsem, wqsem, wosem, osem,
            *, bb, sq, rep, dh, nh, nb, qscale):
    npb = nh // U
    m = bb * sq
    cw = rep * dh
    ntile = m // LANES
    assert npb >= 4 and npb & (npb - 1) == 0 and nb >= 2

    def start_kv(blk, hp, slot):
        for u in range(U):
            for t, hbm in enumerate((k_hbm, v_hbm)):
                pltpu.make_async_copy(
                    hbm.at[pl.ds(blk * bb, bb), hp * U + u], kvbuf.at[slot, t, u],
                    kvsem.at[slot]).start()

    def wait_kv(slot):
        pltpu.make_async_copy(kvbuf.at[slot], kvbuf.at[slot], kvsem.at[slot]).wait()

    def x_copy(blk):
        slot = blk & 1
        return pltpu.make_async_copy(
            x_hbm.at[pl.ds(blk * m, m)], xbuf.at[slot], xsem.at[slot])

    def x0_copy(half):
        mh = m // 2
        return pltpu.make_async_copy(
            x_hbm.at[pl.ds(half * mh, mh)], xbuf.at[0, pl.ds(half * mh, mh)],
            x0sem.at[half])

    def wq_copy(h):
        return pltpu.make_async_copy(
            wq_hbm.at[:, pl.ds(h * cw, cw)], wqbuf.at[h], wqsem.at[h])

    def wo_copy(h):
        return pltpu.make_async_copy(
            wot_hbm.at[:, pl.ds(h * cw, cw)], wobuf.at[h], wosem.at[h])

    def tile_out(blk, t, buf):
        return pltpu.make_async_copy(
            obuf.at[buf, pl.ds(t * LANES, LANES)],
            out_hbm.at[pl.ds(blk * m + t * LANES, LANES)], osem.at[0])

    def wait_out():
        pltpu.make_async_copy(obuf.at[0], out_hbm.at[pl.ds(0, m)], osem.at[0]).wait()

    def project(x, w):
        q = jnp.dot(x, w, preferred_element_type=jnp.float32)
        return (q * qscale).astype(qbuf.dtype)

    x0_copy(0).start()
    wq_copy(0).start()
    x0_copy(1).start()
    wq_copy(1).start()
    acc_ref[...] = jnp.zeros_like(acc_ref)
    x0_copy(0).wait()
    wq_copy(0).wait()
    for h in range(U, nh):
        wq_copy(h).start()
    start_kv(0, 0, 0)
    for u in range(U):
        wo_copy(u).start()
    x_copy(1).start()
    qbuf[0, :m // 2] = project(xbuf[0, :m // 2], wqbuf[0])
    x0_copy(1).wait()
    wq_copy(1).wait()
    qbuf[0, m // 2:] = project(xbuf[0, m // 2:], wqbuf[0])
    qbuf[1] = project(xbuf[0], wqbuf[1])

    def first_projection(p, carry):
        for u in range(U):
            wq_copy(p * U + u).wait()
        wq_pair = wqbuf.at[pl.ds(p * U, U)]
        q_pair = qbuf.at[pl.ds(p * U, U)]
        for u in range(U):
            q_pair[u] = project(xbuf[0], wq_pair[u])
        return carry

    lax.fori_loop(1, npb, first_projection, 0)

    def step(g, last_block):
        if last_block:
            bi = nb - 1
            hp = g
        else:
            bi = lax.shift_right_logical(g, npb.bit_length() - 1)
            hp = g & (npb - 1)
        slot = hp & 1
        first_pair = hp == 0
        last_pair = hp == npb - 1

        if not last_block:
            @pl.when(bi == 0)
            def _():
                for u in range(U):
                    wo_copy(hp * U + u).wait()

            @pl.when(first_pair)
            def _():
                x_copy(bi + 1).wait()

        @pl.when(jnp.logical_and(hp == 2, bi > 0))
        def _():
            wait_out()
        wait_kv(slot)

        def prefetch():
            nblk = jnp.where(last_pair, bi + 1, bi)
            nhp = jnp.where(last_pair, 0, hp + 1)

            @pl.when(nblk < nb)
            def _():
                start_kv(nblk, nhp, 1 - slot)

            if not last_block:
                @pl.when(jnp.logical_and(bi == 0, hp + 1 < npb))
                def _():
                    for u in range(U):
                        wo_copy((hp + 1) * U + u).start()

                @pl.when(jnp.logical_and(first_pair, bi + 2 < nb))
                def _():
                    x_copy(bi + 2).start()

        wq_pair = wqbuf.at[pl.ds(hp * U, U)]
        wo_pair = wobuf.at[pl.ds(hp * U, U)]
        q_pair = qbuf.at[pl.ds(hp * U, U)]
        k_all = kvbuf.at[slot, 0]
        v_all = kvbuf.at[slot, 1]

        def qk(u, b):
            q2 = jnp.concatenate(
                [q_pair[u, b * sq:(b + 1) * sq, r * dh:(r + 1) * dh]
                 for r in range(rep)], axis=0)
            return lax.dot_general(q2, k_all[u, b], NT,
                                   preferred_element_type=jnp.float32)

        def pv(u, b, s):
            mx = jnp.max(s, axis=-1, keepdims=True)
            p = jnp.exp2((s - mx) * LOG2E)
            l = jnp.sum(p, axis=-1, keepdims=True)
            o = jnp.dot(p.astype(jnp.bfloat16), v_all[u, b],
                        preferred_element_type=jnp.float32)
            o = o * pl.reciprocal(l, approx=False, full_range=False)
            o = o.astype(jnp.bfloat16)
            return jnp.concatenate([o[r * sq:(r + 1) * sq] for r in range(rep)], axis=1)

        scores = {}
        outs = {}

        def rows(u, lo, hi):
            parts = []
            for b in range(lo // sq, (hi - 1) // sq + 1):
                a = max(lo, b * sq) - b * sq
                e = min(hi, (b + 1) * sq) - b * sq
                parts.append(outs[u, b][a:e])
            return parts[0] if len(parts) == 1 else jnp.concatenate(parts, axis=0)

        def oproj(u, j):
            lo, hi = j * LANES, (j + 1) * LANES
            prev = acc_ref[j]
            if u == 0:
                obuf[slot, lo:hi, :] = prev.T.astype(obuf.dtype)

                @pl.when(jnp.logical_and(first_pair, bi > 0))
                def _():
                    tile_out(bi - 1, j, 0).start()
                prev = jnp.where(first_pair, 0.0, prev)
            new = prev + lax.dot_general(wo_pair[u], rows(u, lo, hi), NT,
                                         preferred_element_type=jnp.float32)
            acc_ref[j] = new
            if last_block and u == U - 1 and j < ntile - 1:
                obuf[2, lo:hi, :] = new.T.astype(obuf.dtype)

                @pl.when(last_pair)
                def _():
                    tile_out(nb - 1, j, 2).start()

        for op in _schedule(bb, sq, ntile, last_block):
            if op[0] == "qk":
                scores[op[1:]] = qk(*op[1:])
            elif op[0] == "pv":
                outs[op[1:]] = pv(*op[1:], scores.pop(op[1:]))
            elif op[0] == "out":
                oproj(*op[1:])
            elif op[0] == "project":
                q_pair[op[1]] = project(xbuf[(bi + 1) & 1], wq_pair[op[1]])
            else:
                prefetch()

    def inner_step(g, carry):
        step(g, False)
        return carry

    def last_block_step(g, carry):
        step(g, True)
        return carry

    lax.fori_loop(0, (nb - 1) * npb, inner_step, 0)
    lax.fori_loop(0, npb, last_block_step, 0)

    t = ntile - 1
    obuf[2, t * LANES:(t + 1) * LANES, :] = acc_ref[t].T.astype(obuf.dtype)
    tile_out(nb - 1, t, 2).start()
    wait_out()


@jax.jit
def pallas_standalone__gqa_block_cached__near_ridge_kernel(
    x: jax.Array,
    k_cache: jax.Array,
    v_cache: jax.Array,
    wq: jax.Array,
    wo: jax.Array,
):
    B, Sq, D = x.shape
    _, Hkv, Sk, Dh = k_cache.shape
    Hq = wq.shape[1] // Dh
    rep = Hq // Hkv
    bb = 8
    nb = B // bb
    m = bb * Sq
    cw = rep * Dh
    assert B % bb == 0 and m % LANES == 0 and Hkv % U == 0
    qscale = Dh ** -0.5

    kernel = functools.partial(_kernel, bb=bb, sq=Sq, rep=rep, dh=Dh, nh=Hkv, nb=nb,
                               qscale=qscale)
    hbm = pl.BlockSpec(memory_space=pltpu.HBM)
    out = pl.pallas_call(
        kernel,
        in_specs=[hbm] * 5,
        out_specs=hbm,
        out_shape=jax.ShapeDtypeStruct((B * Sq, D), x.dtype),
        scratch_shapes=[
            pltpu.VMEM((2, m, D), x.dtype),
            pltpu.VMEM((2, 2, U, bb, Sk, Dh), k_cache.dtype),
            pltpu.VMEM((Hkv, D, cw), wq.dtype),
            pltpu.VMEM((Hkv, D, cw), wo.dtype),
            pltpu.VMEM((Hkv, m, cw), x.dtype),
            pltpu.VMEM((m // LANES, D, LANES), jnp.float32),
            pltpu.VMEM((3, m, D), x.dtype),
            pltpu.SemaphoreType.DMA((2,)),
            pltpu.SemaphoreType.DMA((2,)),
            pltpu.SemaphoreType.DMA((2,)),
            pltpu.SemaphoreType.DMA((Hkv,)),
            pltpu.SemaphoreType.DMA((Hkv,)),
            pltpu.SemaphoreType.DMA((1,)),
        ],
        compiler_params=pltpu.CompilerParams(
            vmem_limit_bytes=100 * 1024 * 1024,
            disable_bounds_checks=True,
            disable_semaphore_checks=True,
        ),
    )(x.reshape(B * Sq, D), k_cache, v_cache, wq, wo.T)
    return out.reshape(B, Sq, D)
```

```python
import functools

import jax
import jax.numpy as jnp
from jax import lax
import jax.experimental.pallas as pl
import jax.experimental.pallas.tpu as pltpu

U = 4
HOSTED = 2
PRO = 3
LANES = 128
LOG2E = 1.4426950408889634
NT = (((1,), (1,)), ((), ()))


def _schedule(bb, sq, ntile):
    lag = 2
    n = U * bb
    ops = [("load_q", 0, 0)]
    ops += [("project", t) for t in range(HOSTED)]
    ops.append(("qk", 0, 0))
    todo = [(u, j) for u in range(U) for j in range(ntile)]
    for i in range(n):
        u, b = divmod(i, bb)
        if i + 1 < n:
            ops.append(("qk",) + divmod(i + 1, bb))
        if i == 1:
            ops.append(("prefetch",))
        ops.append(("pv", u, b))
        while todo:
            tu, tj = todo[0]
            last_producer = tu * bb + ((tj + 1) * LANES - 1) // sq
            if last_producer + lag > i and i < n - 1:
                break
            ops.append(("out", tu, tj))
            todo.pop(0)
    return ops


def _kernel(x_hbm, k_hbm, v_hbm, wq_hbm, wot_hbm, out_hbm,
            xbuf, kvbuf, wqbuf, wobuf, qbuf, acc_ref, obuf,
            xsem, x0sem, kvsem, wqsem, wosem, osem,
            *, bb, sq, rep, dh, nh, nb, qscale):
    nsteps = nb * nh // U
    m = bb * sq
    cw = rep * dh
    ntile = m // LANES
    npro = nb * nh - HOSTED * nsteps
    assert nh == 2 * U == 8 and nb == 4 and npro == 2 * nh and (npro - 1) % PRO == 0

    def start_kv(s, slot):
        for u in range(U):
            for t, hbm in enumerate((k_hbm, v_hbm)):
                pltpu.make_async_copy(
                    hbm.at[pl.ds((s >> 1) * bb, bb), (s & 1) * U + u], kvbuf.at[slot, t, u],
                    kvsem.at[slot]).start()

    def wait_kv(slot):
        pltpu.make_async_copy(kvbuf.at[slot], kvbuf.at[slot], kvsem.at[slot]).wait()

    def x_copy(blk):
        return pltpu.make_async_copy(
            x_hbm.at[pl.ds(blk * m, m)], xbuf.at[blk], xsem.at[blk])

    def x0_copy(half):
        mh = m // 2
        return pltpu.make_async_copy(
            x_hbm.at[pl.ds(half * mh, mh)], xbuf.at[0, pl.ds(half * mh, mh)],
            x0sem.at[half])

    def wq_copy(h):
        return pltpu.make_async_copy(
            wq_hbm.at[:, pl.ds(h * cw, cw)], wqbuf.at[h], wqsem.at[h])

    def wo_copy(h):
        return pltpu.make_async_copy(
            wot_hbm.at[:, pl.ds(h * cw, cw)], wobuf.at[h], wosem.at[h])

    def tile_out(blk, t, buf):
        return pltpu.make_async_copy(
            obuf.at[buf, pl.ds(t * LANES, LANES)],
            out_hbm.at[pl.ds(blk * m + t * LANES, LANES)], osem.at[0])

    def wait_out():
        pltpu.make_async_copy(obuf.at[0], out_hbm.at[pl.ds(0, m)], osem.at[0]).wait()

    def project(x, w):
        q = jnp.dot(x, w, preferred_element_type=jnp.float32)
        return (q * qscale).astype(qbuf.dtype)

    x0_copy(0).start()
    wq_copy(0).start()
    x0_copy(1).start()
    acc_ref[...] = jnp.zeros_like(acc_ref)
    x0_copy(0).wait()
    wq_copy(0).wait()
    for h in range(1, nh):
        wq_copy(h).start()
    x_copy(1).start()
    start_kv(0, 0)
    for u in range(U):
        wo_copy(u).start()
    x_copy(2).start()
    x_copy(3).start()
    qbuf[0, :m // 2] = project(xbuf[0, :m // 2], wqbuf[0])
    x0_copy(1).wait()
    qbuf[0, m // 2:] = project(xbuf[0, m // 2:], wqbuf[0])

    def first_projections(p, carry):
        k0 = 1 + p * PRO
        for t in range(PRO):
            @pl.when(k0 + t < nh)
            def _():
                wq_copy(k0 + t).wait()

            @pl.when(k0 + t == nh)
            def _():
                x_copy(1).wait()

        q_grp = qbuf.at[pl.ds(k0, PRO)]
        for t in range(PRO):
            k = k0 + t
            q_grp[t] = project(xbuf[lax.shift_right_logical(k, 3)], wqbuf[k & (nh - 1)])
        return carry

    lax.fori_loop(0, (npro - 1) // PRO, first_projections, 0)

    def step(s, carry):
        bi = lax.shift_right_logical(s, 1)
        half = s & 1
        slot = half
        first_half = half == 0
        last_step = s == nsteps - 1

        @pl.when(bi == 0)
        def _():
            for u in range(U):
                wo_copy(half * U + u).wait()

        @pl.when(s == 0)
        def _():
            x_copy(2).wait()

        @pl.when(s == 4)
        def _():
            x_copy(3).wait()

        @pl.when(jnp.logical_and(first_half, bi > 1))
        def _():
            wait_out()
        wait_kv(slot)

        def prefetch():
            @pl.when(s + 1 < nsteps)
            def _():
                start_kv(s + 1, 1 - slot)

            @pl.when(s == 0)
            def _():
                for u in range(U):
                    wo_copy(U + u).start()

        oslot = jnp.where(first_half, 0, jnp.where(last_step, 2, 1))
        send_prev = jnp.logical_and(first_half, bi > 0)
        k0 = npro + s * HOSTED
        x_host = xbuf.at[lax.shift_right_logical(k0, 3)]
        wq_host = wqbuf.at[pl.ds(k0 & (nh - 1), HOSTED)]
        q_host = qbuf.at[pl.ds(k0, HOSTED)]
        q_grp = qbuf.at[pl.ds(s * U, U)]
        wo_grp = wobuf.at[pl.ds(half * U, U)]
        k_all = kvbuf.at[slot, 0]
        v_all = kvbuf.at[slot, 1]

        preloaded = {}
        scores = {}
        outs = {}
        finished = {}

        def load_q(u, b):
            return jnp.concatenate(
                [q_grp[u, b * sq:(b + 1) * sq, r * dh:(r + 1) * dh]
                 for r in range(rep)], axis=0)

        def qk(u, b):
            q2 = preloaded.pop((u, b)) if (u, b) in preloaded else load_q(u, b)
            return lax.dot_general(q2, k_all[u, b], NT,
                                   preferred_element_type=jnp.float32)

        def pv(u, b, sc):
            mx = jnp.max(sc, axis=-1, keepdims=True)
            p = jnp.exp2((sc - mx) * LOG2E)
            l = jnp.sum(p, axis=-1, keepdims=True)
            o = jnp.dot(p.astype(jnp.bfloat16), v_all[u, b],
                        preferred_element_type=jnp.float32)
            o = o * pl.reciprocal(l, approx=False, full_range=False)
            o = o.astype(jnp.bfloat16)
            return jnp.concatenate([o[r * sq:(r + 1) * sq] for r in range(rep)], axis=1)

        def rows(u, lo, hi):
            parts = []
            for b in range(lo // sq, (hi - 1) // sq + 1):
                a = max(lo, b * sq) - b * sq
                e = min(hi, (b + 1) * sq) - b * sq
                parts.append(outs[u, b][a:e])
            return parts[0] if len(parts) == 1 else jnp.concatenate(parts, axis=0)

        def send(cond, blk, j, buf):
            @pl.when(cond)
            def _():
                tile_out(blk, j, buf).start()

        def oproj(u, j):
            lo, hi = j * LANES, (j + 1) * LANES
            merged = j < ntile - 1
            prev = acc_ref[j]
            if u == 0:
                if merged:
                    finished[j] = prev
                else:
                    obuf[oslot, lo:hi, :] = prev.T.astype(obuf.dtype)
                    send(send_prev, bi - 1, j, 0)
                prev = jnp.where(first_half, 0.0, prev)
            new = prev + lax.dot_general(wo_grp[u], rows(u, lo, hi), NT,
                                         preferred_element_type=jnp.float32)
            acc_ref[j] = new
            if merged and u == U - 1:
                val = jnp.where(last_step, new, finished[j])
                obuf[oslot, lo:hi, :] = val.T.astype(obuf.dtype)
                send(send_prev, bi - 1, j, 0)
                send(last_step, bi, j, 2)

        for op in _schedule(bb, sq, ntile):
            if op[0] == "load_q":
                preloaded[op[1:]] = load_q(*op[1:])
            elif op[0] == "project":
                q_host[op[1]] = project(x_host[...], wq_host[op[1]])
            elif op[0] == "qk":
                scores[op[1:]] = qk(*op[1:])
            elif op[0] == "pv":
                outs[op[1:]] = pv(*op[1:], scores.pop(op[1:]))
            elif op[0] == "out":
                oproj(*op[1:])
            else:
                prefetch()
        return carry

    lax.fori_loop(0, nsteps, step, 0)

    t = ntile - 1
    obuf[2, t * LANES:(t + 1) * LANES, :] = acc_ref[t].T.astype(obuf.dtype)
    tile_out(nb - 1, t, 2).start()
    wait_out()
    wait_out()


@jax.jit
def pallas_standalone__gqa_block_cached__near_ridge_kernel(
    x: jax.Array,
    k_cache: jax.Array,
    v_cache: jax.Array,
    wq: jax.Array,
    wo: jax.Array,
):
    B, Sq, D = x.shape
    _, Hkv, Sk, Dh = k_cache.shape
    Hq = wq.shape[1] // Dh
    rep = Hq // Hkv
    bb = 8
    nb = B // bb
    m = bb * Sq
    cw = rep * Dh
    assert B % bb == 0 and m % LANES == 0
    qscale = Dh ** -0.5

    kernel = functools.partial(_kernel, bb=bb, sq=Sq, rep=rep, dh=Dh, nh=Hkv, nb=nb,
                               qscale=qscale)
    hbm = pl.BlockSpec(memory_space=pltpu.HBM)
    out = pl.pallas_call(
        kernel,
        in_specs=[hbm] * 5,
        out_specs=hbm,
        out_shape=jax.ShapeDtypeStruct((B * Sq, D), x.dtype),
        scratch_shapes=[
            pltpu.VMEM((nb, m, D), x.dtype),
            pltpu.VMEM((2, 2, U, bb, Sk, Dh), k_cache.dtype),
            pltpu.VMEM((Hkv, D, cw), wq.dtype),
            pltpu.VMEM((Hkv, D, cw), wo.dtype),
            pltpu.VMEM((nb * Hkv, m, cw), x.dtype),
            pltpu.VMEM((m // LANES, D, LANES), jnp.float32),
            pltpu.VMEM((3, m, D), x.dtype),
            pltpu.SemaphoreType.DMA((nb,)),
            pltpu.SemaphoreType.DMA((2,)),
            pltpu.SemaphoreType.DMA((2,)),
            pltpu.SemaphoreType.DMA((Hkv,)),
            pltpu.SemaphoreType.DMA((Hkv,)),
            pltpu.SemaphoreType.DMA((1,)),
        ],
        compiler_params=pltpu.CompilerParams(
            vmem_limit_bytes=110 * 1024 * 1024,
            disable_bounds_checks=True,
            disable_semaphore_checks=True,
        ),
    )(x.reshape(B * Sq, D), k_cache, v_cache, wq, wo.T)
    return out.reshape(B, Sq, D)
```
